```python
import jax
import jax.numpy as jnp

def _softmax(x, axis=-1):
    return jax.nn.softmax(x, axis=axis)
def _gelu(x):
    return jax.nn.gelu(x, approximate=True)
def _silu(x):
    return jax.nn.silu(x)
def _sigmoid(x):
    return jax.nn.sigmoid(x)
def _layernorm(x, axis=-1, eps=1e-5):
    m = jnp.mean(x, axis=axis, keepdims=True)
    v = jnp.var(x, axis=axis, keepdims=True)
    return (x - m) / jnp.sqrt(v + eps)
def _scatter_add(tgt, idx, src, axis=0):
    return tgt.at[idx].add(src)
def _segment_sum(src, seg, n):
    return jax.ops.segment_sum(src, seg, n)
class _Rng:
    def __init__(self, key):
        self._k = key
    def _next(self):
        self._k, sub = jax.random.split(self._k)
        return sub
    def normal(self, shape):
        return jax.random.normal(self._next(), shape, dtype=jnp.bfloat16)
    def randint(self, lo, hi, shape):
        return jax.random.randint(self._next(), shape, lo, hi, dtype=jnp.int32)
    def uniform(self, shape, lo=0.0, hi=1.0):
        return jax.random.uniform(self._next(), shape, jnp.bfloat16, lo, hi)
    def permutation(self, n):
        return jax.random.permutation(self._next(), n)


kernel_name = 'interleave_layers__sliding_block__moe_arch_mod__prompt'

def setup_inputs():
    _rng = _Rng(jax.random.key(int.from_bytes(__import__("os").urandom(4), "little")))
    _w = (lambda a: (lambda t: t.astype(jnp.bfloat16) if jnp.issubdtype(t.dtype, jnp.floating) else t)(jnp.asarray(a)))
    def _A_setup():
        B, S, D = 1, 2048, 1024
        return {
            "x": _w((lambda *s: _rng.normal(s) * 0.05)(B, S, D)),
            "wqkv": _w((lambda *s: _rng.normal(s) * 0.05)(D, 3 * D)),
            "wo": _w((lambda *s: _rng.normal(s) * 0.05)(D, D)),
        }
    _A_in = _A_setup()

    def _B_setup():
        B, S, D, F, C = 1, 2048, 1024, 3584, 1
        return {
            "x": _w((lambda *s: _rng.normal(s) * 0.05)(B, S, D)),
            "w_r": _w((lambda *s: _rng.normal(s) * 0.05)(D)),
            "w_gate": _w((lambda *s: _rng.normal(s) * 0.05)(D, F)),
            "w_up": _w((lambda *s: _rng.normal(s) * 0.05)(D, F)),
            "w_down": _w((lambda *s: _rng.normal(s) * 0.05)(F, D)),
        }
    _B_in = _B_setup()

    return {
        "A_x": _A_in["x"],
        "A_wqkv": _A_in["wqkv"],
        "A_wo": _A_in["wo"],
        "B_x": _B_in["x"],
        "B_w_r": _B_in["w_r"],
        "B_w_gate": _B_in["w_gate"],
        "B_w_up": _B_in["w_up"],
        "B_w_down": _B_in["w_down"],
    }

def reference(A_x, A_wqkv, A_wo, B_x, B_w_r, B_w_gate, B_w_up, B_w_down):
    def _A_ref(x, wqkv, wo):
        B, S, D = x.shape
        H = 32; Dh = D // H; W = 256
        qkv = (lambda x, *d: x.transpose(*d))((x @ wqkv).reshape(B, S, 3, H, Dh), 2, 0, 3, 1, 4)
        q, k, v = qkv[0], qkv[1], qkv[2]
        scores = jnp.einsum("bhqd,bhkd->bhqk", q, k) * (Dh ** -0.5)
        idx = jnp.arange(S)
        mask = (idx[:, None] - idx[None, :] >= 0) & (idx[:, None] - idx[None, :] < W)
        scores = jnp.where(mask[None, None], scores, -1e9)
        p = _softmax(scores, axis=-1)
        o = jnp.einsum("bhqk,bhkd->bhqd", p, v)
        return (lambda x, *d: x.transpose(*d))(o, 0, 2, 1, 3).reshape(B, S, D) @ wo

    def _B_ref(x, w_r, w_gate, w_up, w_down):
        B, S, D = x.shape
        C = 1
        r = x @ w_r
        idx = jnp.argsort(-r, axis=-1)[:, :C]
        idx_e = jnp.repeat(idx.reshape(B, C, 1), D, axis=2)
        x_sel = jnp.take_along_axis(x, idx_e, axis=1)
        g = _silu(x_sel @ w_gate)
        u = x_sel @ w_up
        y = (g * u) @ w_down
        r_sel = _sigmoid(jnp.take_along_axis(r, idx, axis=1))
        y = y * r_sel.reshape(B, C, 1)
        b_off = (jnp.arange(B) * S).reshape(B, 1)
        flat_idx = (idx + b_off).reshape(B * C)
        zero = (x * 0.0).reshape(B * S, D)
        upd = _scatter_add(zero, flat_idx, y.reshape(B * C, D), axis=0)
        return x + upd.reshape(B, S, D)

    x = A_x
    x = x + _A_ref(_layernorm(x, axis=-1), A_wqkv, A_wo)
    x = x + _B_ref(_layernorm(x, axis=-1), B_w_r, B_w_gate, B_w_up, B_w_down)
    x = x + _A_ref(_layernorm(x, axis=-1), A_wqkv, A_wo)
    x = x + _B_ref(_layernorm(x, axis=-1), B_w_r, B_w_gate, B_w_up, B_w_down)
    return x
```

```python
import functools
import math

import jax
import jax.numpy as jnp
import numpy as np
from jax import lax
from jax.experimental import pallas as pl
from jax.experimental.pallas import tpu as pltpu

S = 2048
D = 1024
F = 3584
NH = 32
DH = D // NH
W = 256
T = 256
NB = S // T
NG = D // 128
CW = 256
EPS = float(np.float32(1e-5).astype(jnp.bfloat16))
LOG2E = math.log2(math.e)
QSCALE = float(np.float32(DH ** -0.5).astype(jnp.bfloat16)) * LOG2E
NEG = -1e9 * LOG2E

F32 = jnp.float32
BF16 = jnp.bfloat16
U32 = jnp.uint32
NT_DIMS = (((1,), (1,)), ((), ()))


def _dot(a, b):
    return jnp.dot(a, b, preferred_element_type=F32)


def _dot_nt(a, b):
    return lax.dot_general(a, b, NT_DIMS, preferred_element_type=F32)


def _round(x):
    return x.astype(BF16).astype(F32)


def _layernorm(x):
    m = jnp.mean(x, axis=-1, keepdims=True)
    mb = _round(m)
    d = x - mb
    v = jnp.mean(d * d, axis=-1, keepdims=True) - (m - mb) * (m - mb)
    sd = _round(jnp.sqrt(_round(_round(jnp.maximum(v, 0.0)) + EPS)))
    return (_round(d) * (1.0 / sd)).astype(BF16)


def _pack(x):
    return pltpu.bitcast(x, U32)


def _unpack(x):
    return pltpu.bitcast(x, BF16)


def _lane_group(shape):
    return lax.broadcasted_iota(jnp.int32, shape, len(shape) - 1) // DH


def _pick(m, a, b):
    if a is None and b is None:
        return None
    z = jnp.zeros_like(a if a is not None else b)
    return jnp.where(m, a if a is not None else z, b if b is not None else z)


def _regroup(vals, grp):
    st = [_pick(grp % 2 == 0, vals[u], vals[(u + 1) % 4]) for u in range(4)]
    return [_pick(grp < 2, st[(-h) % 4], st[(2 - h) % 4]) for h in range(4)]


def _kernel(x_hbm, wqkv_hbm, wo_hbm, wr_ref, wg_hbm, wu_hbm, wd_hbm, out_hbm,
            xs, wqkv, wvt, wo, wg, wu, wd, hbuf, qnew, qcur, kwin, vwin, onew, ocur, x1buf, h2buf,
            bestv, besti, sem_x, sem_w, sem_o):

    def block_rows(i):
        return pl.ds(pl.multiple_of(i * T, T), T)

    def x_copy(i):
        return pltpu.make_async_copy(x_hbm.at[block_rows(i)], xs.at[block_rows(i)], sem_x.at[i])

    def out_copy(i):
        return pltpu.make_async_copy(xs.at[block_rows(i)], out_hbm.at[block_rows(i)], sem_o.at[i])

    w_copies = [pltpu.make_async_copy(src, dst, sem_w.at[n]) for n, (src, dst) in enumerate(
        [(wqkv_hbm, wqkv), (wo_hbm, wo), (wg_hbm, wg), (wu_hbm, wu), (wd_hbm, wd)])]

    x_copy(0).start()
    w_copies[0].start()
    x_copy(1).start()
    w_copies[1].start()
    for i in range(2, NB):
        x_copy(i).start()
    for c in w_copies[2:]:
        c.start()

    w_copies[0].wait()
    for a in range(D // 128):
        wvt[:, a * 128:(a + 1) * 128] = _pack(wqkv[a * 128:(a + 1) * 128, 2 * D:3 * D].T)
    w_copies[1].wait()

    def qkv_chunks(i):
        hbuf[...] = _pack(_layernorm(xs[block_rows(i), :].astype(F32)))

        def q_chunk(c):
            cols = slice(c * CW, (c + 1) * CW)
            qnew[:, cols] = _pack((_dot(_unpack(hbuf[...]), wqkv[:, cols]) * QSCALE).astype(BF16))

        def k_chunk(c):
            cols = slice(c * CW, (c + 1) * CW)
            kwin[T:, cols] = _pack(_dot(_unpack(hbuf[...]), wqkv[:, D + c * CW:D + (c + 1) * CW]).astype(BF16))

        def v_chunk(c):
            rows = slice(c * CW // 2, (c + 1) * CW // 2)
            vwin[rows, 2 * T:] = _pack(_dot_nt(_unpack(wvt[rows, :]), _unpack(hbuf[...])).astype(BF16))

        return [functools.partial(f, c) for f in (q_chunk, k_chunk, v_chunk) for c in range(D // CW)]

    def out_chunks(i):
        rows = block_rows(i)
        ocur[...] = onew[...]

        def chunk(c):
            cols = slice(c * CW, (c + 1) * CW)
            x1buf[:, cols] = xs[rows, cols].astype(F32) + _dot(_unpack(ocur[...]), wo[:, cols])
            if c == D // CW - 1:
                finish()

        def finish():
            x1 = x1buf[...]
            h2 = _layernorm(x1)
            h2buf[pl.ds(pl.multiple_of(i * (T // 2), T // 2), T // 2), :] = _pack(h2)
            h2 = h2.astype(F32)
            xs[rows, :] = (x1 + h2).astype(BF16)
            r = _round(jnp.sum(h2 * wr_ref[...].astype(F32).reshape(1, D), axis=-1, keepdims=True))
            bv, bi = bestv[...], besti[...]
            sub = lax.broadcasted_iota(jnp.int32, (8, 128), 0) + i * T
            for a in range(T // 8):
                ra = jnp.broadcast_to(r[a * 8:(a + 1) * 8], (8, 128))
                better = ra > bv
                bv = jnp.where(better, ra, bv)
                bi = jnp.where(better, sub + a * 8, bi)
            bestv[...] = bv
            besti[...] = bi

        return [functools.partial(chunk, c) for c in range(D // CW)]

    def scores(b, g, first_keys):
        lanes = slice(g * 128, (g + 1) * 128)
        if b == 0:
            drows = slice(g * 64, (g + 1) * 64)
            qcur[:, lanes] = qnew[:, lanes]
            if not first_keys:
                kwin[0:T // 2, lanes] = kwin[T // 2:T, lanes]
                vwin[drows, 0:T] = vwin[drows, T:2 * T]
            kwin[T // 2:T, lanes] = kwin[T:, lanes]
            vwin[drows, T:2 * T] = vwin[drows, 2 * T:]
        grp = _lane_group((DH // 2, 128))
        out = []
        for j in range(4):
            q = qcur[(b * 128 + j * DH) // 2:(b * 128 + (j + 1) * DH) // 2, lanes]
            qbd = jnp.concatenate(
                [jnp.where(grp == (c - j) % 4, q, jnp.zeros_like(q)) for c in range(4)], axis=0)
            lo = max(j, first_keys)
            hi = j + W // DH + 1
            base = T - W + b * 128
            k = kwin[(base + lo * DH) // 2:(base + hi * DH) // 2, lanes]
            out.append((lo, _dot_nt(_unpack(k), _unpack(qbd))))
        return out

    def softmax(ss, first_keys):
        row = lax.broadcasted_iota(jnp.int32, (DH, 128), 0)
        col = lax.broadcasted_iota(jnp.int32, (DH, 128), 1) % DH
        probs, sums = [], []
        for j, (lo, s) in enumerate(ss):
            n = s.shape[0] // DH
            parts = [s[a * DH:(a + 1) * DH] for a in range(n)]
            if lo == j:
                parts[0] = jnp.where(row > col, parts[0], NEG)
            parts[-1] = jnp.where(row <= col, parts[-1], NEG)
            s = jnp.concatenate(parts, axis=0)
            e = jnp.exp2(s - jnp.max(s, axis=0, keepdims=True))
            sums.append(jnp.sum(e, axis=0, keepdims=True))
            e = _pack(e.astype(BF16))
            probs.append({lo + a: e[a * DH // 2:(a + 1) * DH // 2] for a in range(n)})
        grp = _lane_group((DH // 2, 128))
        per_head = [[] for _ in range(4)]
        for a in range(first_keys // 4 * 4, 12):
            for h, v in enumerate(_regroup([probs[j].get(a) for j in range(4)], grp)):
                per_head[h].append(v)
        inv = _regroup([1.0 / v for v in sums], _lane_group((1, 128)))
        return [_unpack(jnp.concatenate(p, axis=0)) for p in per_head], inv

    def values(b, g, first_keys, ps, inv):
        outs = []
        k0 = T - W + b * 128
        for h in range(4):
            drows = slice((g * 4 + h) * DH // 2, (g * 4 + h + 1) * DH // 2)
            vt = _unpack(vwin[drows, k0 + first_keys // 4 * 128:k0 + W + 128])
            o = _dot(vt, ps[h]) * inv[h]
            outs.append(pltpu.roll(o, (128 - DH * h) % 128, axis=1) if h else o)
        ot = jnp.concatenate(outs, axis=0)
        onew[b * 64:(b + 1) * 64, g * 128:(g + 1) * 128] = _pack(ot.T.astype(BF16))

    def step(attn, qkv, out, first=False):
        pre = out_chunks(out) if out is not None else []
        post = qkv_chunks(qkv) if qkv is not None else []
        if not attn:
            for f in pre + post:
                f()
            return
        groups = [(b, g, max(0, (W - b * 128) // DH) if first else 0)
                  for b in range(T // 128) for g in range(NG)]
        ng = len(groups)
        slots = [[] for _ in range(ng)]
        if post:
            for n, f in enumerate(pre):
                slots[n].append(f)
            for n, f in enumerate(post):
                slots[ng - len(post) + n].append(f)
        else:
            for n, f in enumerate(pre):
                slots[n * (ng - 3) // len(pre)].append(f)
        ss = scores(*groups[0])
        for n, grp in enumerate(groups):
            nxt = scores(*groups[n + 1]) if n + 1 < ng else None
            ps, inv = softmax(ss, grp[2])
            for f in slots[n]:
                f()
            values(*grp, ps, inv)
            ss = nxt

    def ffn():
        bv, bi = bestv[...], besti[...]
        rmax = jnp.max(bv, axis=0, keepdims=True)
        sel = jnp.min(jnp.where(bv == rmax, bi, S - 1))
        tile = sel // 16
        hs = _unpack(h2buf[pl.ds(pl.multiple_of(tile * 8, 8), 8), :])
        gate = _round(_dot(hs, wg[...]))
        up = _round(_dot(hs, wu[...]))
        act = (_round(gate * jax.nn.sigmoid(gate)) * up).astype(BF16)
        y = _dot(act, wd[...]) * _round(jax.nn.sigmoid(rmax[:, 0:1]))
        hit = lax.broadcasted_iota(jnp.int32, (16, D), 0) + tile * 16 == sel
        return pl.ds(pl.multiple_of(tile * 16, 16), 16), hit, y

    def layer(l, carry):
        bestv[...] = jnp.full((8, 128), -jnp.inf, F32)
        besti[...] = jnp.zeros((8, 128), jnp.int32)

        def need_x(i):
            @pl.when(l == 0)
            def _():
                x_copy(i).wait()

        def emit(i):
            @pl.when(l == 1)
            def _():
                out_copy(i).start()

        need_x(0)
        step(False, 0, None)
        need_x(1)
        step(True, 1, None, first=True)

        def body(i, c):
            need_x(i + 1)
            step(True, i + 1, i - 1)
            emit(i - 1)
            return c

        lax.fori_loop(1, NB - 1, body, 0)
        step(True, None, NB - 2)
        emit(NB - 2)
        step(False, None, NB - 1)
        emit(NB - 1)

        @pl.when(l == 0)
        def _():
            for c in w_copies[2:]:
                c.wait()

        rows, hit, y = ffn()

        @pl.when(l == 1)
        def _():
            for i in range(NB):
                out_copy(i).wait()

        old = xs[rows, :].astype(F32)
        xs[rows, :] = jnp.where(hit, old + y, old).astype(BF16)

        @pl.when(l == 1)
        def _():
            c = pltpu.make_async_copy(xs.at[rows], out_hbm.at[rows], sem_o.at[0])
            c.start()
            c.wait()

        return carry

    lax.fori_loop(0, 2, layer, 0)


@jax.jit
def pallas_interleave_layers__sliding_block__moe_arch_mod__prompt_kernel(
    A_x: jax.Array,
    A_wqkv: jax.Array,
    A_wo: jax.Array,
    B_x: jax.Array,
    B_w_r: jax.Array,
    B_w_gate: jax.Array,
    B_w_up: jax.Array,
    B_w_down: jax.Array,
):
    del B_x
    hbm = pl.BlockSpec(memory_space=pl.ANY)
    out = pl.pallas_call(
        _kernel,
        out_shape=jax.ShapeDtypeStruct((S, D), BF16),
        in_specs=[hbm, hbm, hbm, pl.BlockSpec(memory_space=pltpu.VMEM), hbm, hbm, hbm],
        out_specs=hbm,
        scratch_shapes=[
            pltpu.VMEM((S, D), BF16),
            pltpu.VMEM((D, 3 * D), BF16),
            pltpu.VMEM((D // 2, D), U32),
            pltpu.VMEM((D, D), BF16),
            pltpu.VMEM((D, F), BF16),
            pltpu.VMEM((D, F), BF16),
            pltpu.VMEM((F, D), BF16),
            pltpu.VMEM((T // 2, D), U32),
            pltpu.VMEM((T // 2, D), U32),
            pltpu.VMEM((T // 2, D), U32),
            pltpu.VMEM((3 * T // 2, D), U32),
            pltpu.VMEM((D // 2, 3 * T), U32),
            pltpu.VMEM((T // 2, D), U32),
            pltpu.VMEM((T // 2, D), U32),
            pltpu.VMEM((T, D), F32),
            pltpu.VMEM((S // 2, D), U32),
            pltpu.VMEM((8, 128), F32),
            pltpu.VMEM((8, 128), jnp.int32),
            pltpu.SemaphoreType.DMA((NB,)),
            pltpu.SemaphoreType.DMA((5,)),
            pltpu.SemaphoreType.DMA((NB,)),
        ],
        compiler_params=pltpu.CompilerParams(vmem_limit_bytes=100 * 2 ** 20),
        name="interleave_layers",
    )(A_x.reshape(S, D), A_wqkv, A_wo, B_w_r, B_w_gate, B_w_up, B_w_down)
    return out.reshape(1, S, D)
```

```python
import functools
import itertools
import math

import jax
import jax.numpy as jnp
import numpy as np
from jax import lax
from jax.experimental import pallas as pl
from jax.experimental.pallas import tpu as pltpu

S = 2048
D = 1024
F = 3584
NH = 32
DH = D // NH
W = 256
T = 256
NB = S // T
NG = D // 128
PS = 4
EPS = float(np.float32(1e-5).astype(jnp.bfloat16))
LOG2E = math.log2(math.e)
QSCALE = float(np.float32(DH ** -0.5).astype(jnp.bfloat16)) * LOG2E
NEG = -1e9 * LOG2E

F32 = jnp.float32
BF16 = jnp.bfloat16
U32 = jnp.uint32
NT_DIMS = (((1,), (1,)), ((), ()))


def _dot(a, b):
    return jnp.dot(a, b, preferred_element_type=F32)


def _dot_nt(a, b):
    return lax.dot_general(a, b, NT_DIMS, preferred_element_type=F32)


def _round(x):
    return x.astype(BF16).astype(F32)


def _after(x, tok):
    return x if tok is None else jnp.where(tok < 0.0, tok, x)


def _layernorm(x, tok=None):
    m = _after(jnp.mean(x, axis=-1, keepdims=True), tok)
    mb = _round(m)
    d = x - mb
    v = jnp.mean(d * d, axis=-1, keepdims=True) - (m - mb) * (m - mb)
    v = _round(_round(jnp.maximum(v, 0.0)) + EPS)
    sd = _round(jnp.where(v < jnp.inf, v * lax.rsqrt(v), v))
    inv = lax.rsqrt(sd * sd)
    return (_round(d) * inv).astype(BF16), inv


def _pack(x):
    return pltpu.bitcast(x, U32)


def _unpack(x):
    return pltpu.bitcast(x, BF16)


def _lane_group(shape):
    return lax.broadcasted_iota(jnp.int32, shape, len(shape) - 1) // DH


def _pick(m, a, b):
    if a is None and b is None:
        return None
    z = jnp.zeros_like(a if a is not None else b)
    return jnp.where(m, a if a is not None else z, b if b is not None else z)


def _regroup(vals, grp):
    st = [_pick(grp % 2 == 0, vals[u], vals[(u + 1) % 4]) for u in range(4)]
    return [_pick(grp < 2, st[(-h) % 4], st[(2 - h) % 4]) for h in range(4)]


def _kernel(x_hbm, wqkv_hbm, wo_hbm, wr_ref, wg_hbm, wu_hbm, wd_hbm, out_hbm,
            xs, wqkv, wo, wg, wu, wd, hnew, hbuf, qkbuf, qnew, qcur, kwin, vwin, onew, ocur, x1buf, h2buf,
            pbuf, bestv, besti, sem_x, sem_q, sem_w, sem_o):

    def block_rows(i):
        return pl.ds(pl.multiple_of(i * T, T), T)

    def x_copy(i):
        return pltpu.make_async_copy(x_hbm.at[block_rows(i)], xs.at[block_rows(i)], sem_x.at[i])

    def out_copy(i):
        return pltpu.make_async_copy(xs.at[block_rows(i)], out_hbm.at[block_rows(i)], sem_o.at[i])

    def wqkv_copy(c):
        cols = pl.ds(pl.multiple_of(c * 128, 128), 128)
        return pltpu.make_async_copy(wqkv_hbm.at[:, cols], wqkv.at[c], sem_q.at[c])

    wo_copies = [pltpu.make_async_copy(wo_hbm.at[:, c * 128:(c + 1) * 128], wo.at[c], sem_q.at[3 * NG + c])
                 for c in range(NG)]
    ffn_copies = [pltpu.make_async_copy(src, dst, sem_w.at[n]) for n, (src, dst) in enumerate(
        [(wg_hbm, wg), (wu_hbm, wu), (wd_hbm, wd)])]
    wqkv_p, wo_p, pbuf_p = wqkv.bitcast(U32), wo.bitcast(U32), pbuf.bitcast(U32)

    x_copy(0).start()
    def strip(n):
        if isinstance(n, int):
            return (n + 2 * NG) % (3 * NG)
        return jnp.where(n < NG, n + 2 * NG, n - NG)

    for c in range(PS):
        wqkv_copy(strip(c)).start()

    HK = D // 2

    def fold(v):
        out = v[0:8]
        for a in range(1, v.shape[0] // 8):
            out = jnp.maximum(out, v[a * 8:(a + 1) * 8])
        return out[0:1]

    def norm_piece(i, c, n, tok):
        h, inv = _layernorm(xs[pl.ds(pl.multiple_of(i * T + c * n, n), n), :].astype(F32), tok)
        hnew[c * n // 2:(c + 1) * n // 2, :] = _pack(h)
        return fold(inv)

    def route_piece(i, c, n, tok):
        r0 = i * T + c * n
        rows = pl.ds(pl.multiple_of(r0, n), n)
        x1 = x1buf[c * n:(c + 1) * n, :]
        h2, _ = _layernorm(x1, tok)
        h2buf[pl.ds(pl.multiple_of(r0 // 2, n // 2), n // 2), :] = _pack(h2)
        h2 = h2.astype(F32)
        xs[rows, :] = (x1 + h2).astype(BF16)
        r = _round(jnp.sum(h2 * wr_ref[...].astype(F32).reshape(1, D), axis=-1, keepdims=True))
        bv, bi = bestv[...], besti[...]
        sub = lax.broadcasted_iota(jnp.int32, (8, 128), 0) + r0
        for a in range(n // 8):
            ra = jnp.broadcast_to(r[a * 8:(a + 1) * 8], (8, 128))
            better = ra > bv
            bv = jnp.where(better, ra, bv)
            bi = jnp.where(better, sub + a * 8, bi)
        bestv[...] = bv
        besti[...] = bi
        return jnp.abs(bv[0:1])

    def store_qkv(c, val):
        cols = slice(c % NG * 128, (c % NG + 1) * 128)
        if c < NG:
            qnew[:, cols] = _pack(val)
        elif c < 2 * NG:
            kwin[T:, cols] = _pack(val)
        else:
            vwin[c % NG * 64:(c % NG + 1) * 64, 2 * T:] = _pack(val.T)

    def qkv_rounds(i):
        for c in [*range(NG), *range(2 * NG, 3 * NG), *range(NG, 2 * NG)]:
            acc = _dot(_unpack(hbuf[:, 0:HK]), _unpack(wqkv_p[c, 0:HK // 2]))
            yield jnp.abs(acc[0:1])
            acc = acc + _dot(_unpack(hbuf[:, HK:]), _unpack(wqkv_p[c, HK // 2:]))
            store_qkv(c, (acc * QSCALE if c < NG else acc).astype(BF16))
            yield jnp.abs(acc[0:1])

    def out_rounds(i):
        rows = block_rows(i)
        ocur[...] = onew[...]
        for c in range(NG):
            cols = slice(c * 128, (c + 1) * 128)
            acc = xs[rows, cols].astype(F32) + _dot(_unpack(ocur[:, 0:HK]), _unpack(wo_p[c, 0:HK // 2]))
            yield jnp.abs(acc[0:1])
            x1buf[0:T, cols] = acc + _dot(_unpack(ocur[:, HK:]), _unpack(wo_p[c, HK // 2:]))
            tok = jnp.abs(acc[0:1, 0:1])
            yield tok

    def final_out_rounds(b):
        rows = slice(S - 2 * T + b * 128, S - 2 * T + (b + 1) * 128)
        src = ocur if b < 2 else onew
        tok = None
        for c in range(NG):
            cols = slice(c * 128, (c + 1) * 128)
            o = src[b % 2 * 64:(b % 2 + 1) * 64, :]
            if tok is not None:
                o = jnp.concatenate([jnp.where(tok < 0.0, jnp.uint32(0), o[0:8]), o[8:]], axis=0)
            x1 = xs[rows, cols].astype(F32) + _dot(_unpack(o), _unpack(wo_p[c]))
            x1buf[b * 128:(b + 1) * 128, cols] = x1
            tok = yield jnp.abs(x1[0:1, 0:1])

    def prologue(l):
        def project(c):
            return _dot(_unpack(hbuf[...]), _unpack(wqkv_p[c]))

        @pl.when(l == 0)
        def _():
            x_copy(0).wait()
            for c in range(PS, 2 * PS):
                wqkv_copy(strip(c)).start()

        norm_piece(0, 0, T, None)
        hbuf[...] = hnew[...]
        nloop = 3 * NG // PS - 1

        def part(p, carry):
            @pl.when(l == 0)
            def _():
                for c in range(PS):
                    wqkv_copy(strip(p * PS + c)).wait()

                @pl.when(p < nloop - 1)
                def _():
                    for c in range(PS):
                        wqkv_copy(strip((p + 2) * PS + c)).start()

                @pl.when(p >= nloop - 2)
                def _():
                    x_copy(p - nloop + 3).start()

            for c in range(PS):
                c = strip(p * PS + c)
                scale = jnp.where(c < NG, QSCALE, 1.0)
                qkbuf[:, pl.ds(pl.multiple_of(c * 128, 128), 128)] = _pack((project(c) * scale).astype(BF16))
            return carry

        lax.fori_loop(0, nloop, part, 0)

        @pl.when(l == 0)
        def _():
            for c in range(nloop * PS, 3 * NG):
                wqkv_copy(strip(c)).wait()
            x_copy(1).wait()

        for c in range(nloop * PS):
            store_qkv(strip(c), _unpack(qkbuf[:, strip(c) * 128:(strip(c) + 1) * 128]))
        tok = None
        for n in range(PS):
            val = project(strip(nloop * PS + n))
            store_qkv(strip(nloop * PS + n), val.astype(BF16))
            norm_piece(1, n, T // PS, tok)
            tok = jnp.abs(val[0:1, 0:1])

        @pl.when(l == 0)
        def _():
            x_copy(2).wait()
            x_copy(3).start()
            for c in wo_copies:
                c.start()

    def scores(b, g, first_keys):
        lanes = slice(g * 128, (g + 1) * 128)
        if b == 0:
            drows = slice(g * 64, (g + 1) * 64)
            if not first_keys:
                kwin[0:T // 2, lanes] = kwin[T // 2:T, lanes]
                vwin[drows, 0:T] = vwin[drows, T:2 * T]
            kwin[T // 2:T, lanes] = kwin[T:, lanes]
            vwin[drows, T:2 * T] = vwin[drows, 2 * T:]
        grp = _lane_group((DH // 2, 128))
        out = []
        for j in range(4):
            q = qcur[(b * 128 + j * DH) // 2:(b * 128 + (j + 1) * DH) // 2, lanes]
            qbd = jnp.concatenate(
                [jnp.where(grp == (c - j) % 4, q, jnp.zeros_like(q)) for c in range(4)], axis=0)
            lo = max(j, first_keys)
            hi = j + W // DH + 1
            base = T - W + b * 128
            k = kwin[(base + lo * DH) // 2:(base + hi * DH) // 2, lanes]
            out.append((lo, _dot_nt(_unpack(k), _unpack(qbd))))
        return out

    def softmax(ss, first_keys, tok, slot):
        row = lax.broadcasted_iota(jnp.int32, (DH, 128), 0)
        col = lax.broadcasted_iota(jnp.int32, (DH, 128), 1) % DH
        probs, sums = [], []
        for j, (lo, s) in enumerate(ss):
            n = s.shape[0] // DH
            parts = [s[a * DH:(a + 1) * DH] for a in range(n)]
            if lo == j:
                parts[0] = jnp.where(row > col, parts[0], NEG)
            parts[-1] = jnp.where(row <= col, parts[-1], NEG)
            s = jnp.concatenate(parts, axis=0)
            m = jnp.max(s, axis=0, keepdims=True)
            m = _after(m, sums[-1] if sums else tok)
            e = jnp.exp2(s - m)
            sums.append(jnp.sum(e, axis=0, keepdims=True))
            pbuf[slot * 4 + j, 0:n * DH, :] = e.astype(BF16)
            e = pbuf_p[slot * 4 + j, 0:n * DH // 2, :]
            probs.append({lo + a: e[a * DH // 2:(a + 1) * DH // 2] for a in range(n)})
        grp = _lane_group((DH // 2, 128))
        per_head = [[] for _ in range(4)]
        for a in range(first_keys // 4 * 4, 12):
            for h, v in enumerate(_regroup([probs[j].get(a) for j in range(4)], grp)):
                per_head[h].append(v)
        inv = _regroup([1.0 / v for v in sums], _lane_group((1, 128)))
        return [_unpack(jnp.concatenate(p, axis=0)) for p in per_head], inv, sums[-1]

    def values(b, g, first_keys, ps, inv):
        k0 = T - W + b * 128
        t0 = first_keys // 4
        accs = [None] * 4
        for t in range(3):
            if t >= t0:
                for h in range(4):
                    drows = slice((g * 4 + h) * DH // 2, (g * 4 + h + 1) * DH // 2)
                    vt = _unpack(vwin[drows, k0 + t * 128:k0 + (t + 1) * 128])
                    o = _dot(vt, ps[h][(t - t0) * 128:(t - t0 + 1) * 128])
                    accs[h] = o if accs[h] is None else accs[h] + o
            if t == 2:
                outs = [accs[h] * inv[h] for h in range(4)]
                outs = [pltpu.roll(o, (128 - DH * h) % 128, axis=1) if h else o for h, o in enumerate(outs)]
                ot = jnp.concatenate(outs, axis=0)
                onew[b * 64:(b + 1) * 64, g * 128:(g + 1) * 128] = _pack(ot.T.astype(BF16))
            yield

    def step(i, kind):
        groups = [(b, g, max(0, (W - b * 128) // DH) if kind == "first" else 0)
                  for b in range(T // 128) for g in range(NG)]
        ng = len(groups)
        pieces = [[] for _ in range(ng)]
        if kind == "last":
            ocur[...] = onew[...]
            dense = itertools.chain(*[final_out_rounds(b) for b in range(3)])
            per = [2, 1] * (ng // 2)
            for c, n in enumerate([6, 7, 8, 10, 11, 12, 13, 14]):
                pieces[n].append(functools.partial(route_piece, i - 1, c, 32))
        else:
            hbuf[...] = hnew[...]
            ahead = jnp.minimum(i + 2, NB - 1)
            for c in range(8):
                pieces[c * (2 if kind == "first" else 1)].append(functools.partial(norm_piece, ahead, c, T // 8))
            if kind == "first":
                dense, per = qkv_rounds(i + 1), [3] * ng
            else:
                dense, per = itertools.chain(out_rounds(i - 1), qkv_rounds(i + 1)), [4] * ng
                for c in range(8):
                    pieces[7 + c].append(functools.partial(route_piece, i - 1, c, T // 8))

        qcur[...] = qnew[...]
        ss = scores(*groups[0])
        tok, late = None, []
        for n, grp in enumerate(groups):
            nxt = scores(*groups[n + 1]) if n + 1 < ng else None
            ps, inv, tok = softmax(ss, grp[2], tok, n % 2)
            due, late = late, [f(tok[:, 0:1]) for f in pieces[n]]
            for t in (due if kind == "last" else late):
                tok = jnp.maximum(tok, t)
            pv = values(*grp, ps, inv)
            for t in range(4):
                for _ in range((per[n] * (t + 1) + 3) // 4 - (per[n] * t + 3) // 4):
                    td = next(dense)
                    if t == 0:
                        tok = jnp.maximum(tok, td)
                next(pv, None)
            ss = nxt
        if kind == "last":
            rounds = final_out_rounds(3)
            start, done = [tok[:, 0:1]], [None] * 4
            for c in range(NG):
                start.append(rounds.send(done[c]))
                if c < 4:
                    done.append(route_piece(i - 1, 8 + c, 32, start[c])[:, 0:1])
            route_piece(i - 1, 3, 128, None)

    def ffn():
        bv, bi = bestv[...], besti[...]
        rmax = jnp.max(bv, axis=0, keepdims=True)
        sel = jnp.min(jnp.where(bv == rmax, bi, S - 1))
        tile = sel // 16
        hs = _unpack(h2buf[pl.ds(pl.multiple_of(tile * 8, 8), 8), :])
        y = None
        for c in range(F // 512):
            cols = slice(c * 512, (c + 1) * 512)
            gate = _round(_dot(hs, wg[:, cols]))
            up = _round(_dot(hs, wu[:, cols]))
            act = (_round(gate * jax.nn.sigmoid(gate)) * up).astype(BF16)
            part = jnp.concatenate([_dot(act, wd[cols, a * 128:(a + 1) * 128]) for a in range(NG)], axis=1)
            y = part if y is None else y + part
        y = y * _round(jax.nn.sigmoid(rmax[:, 0:1]))
        hit = lax.broadcasted_iota(jnp.int32, (16, D), 0) + tile * 16 == sel
        return pl.ds(pl.multiple_of(tile * 16, 16), 16), hit, y

    def layer(l, carry):
        bestv[...] = jnp.full((8, 128), -jnp.inf, F32)
        besti[...] = jnp.zeros((8, 128), jnp.int32)

        def emit(i):
            @pl.when(l == 1)
            def _():
                out_copy(i).start()

        prologue(l)
        step(0, "first")

        @pl.when(l == 0)
        def _():
            for c in wo_copies:
                c.wait()
            for i in range(4, NB):
                x_copy(i).start()

        def body(i, c):
            @pl.when(jnp.logical_and(l == 0, i + 2 < NB))
            def _():
                x_copy(i + 2).wait()

            @pl.when(jnp.logical_and(l == 0, i == 2))
            def _():
                for cp in ffn_copies:
                    cp.start()

            step(i, "body")
            emit(i - 1)
            return c

        lax.fori_loop(1, NB - 1, body, 0)
        step(NB - 1, "last")
        emit(NB - 2)
        emit(NB - 1)

        @pl.when(l == 0)
        def _():
            for c in ffn_copies:
                c.wait()

        rows, hit, y = ffn()

        @pl.when(l == 1)
        def _():
            for i in range(NB):
                out_copy(i).wait()

        old = xs[rows, :].astype(F32)
        xs[rows, :] = jnp.where(hit, old + y, old).astype(BF16)

        @pl.when(l == 1)
        def _():
            c = pltpu.make_async_copy(xs.at[rows], out_hbm.at[rows], sem_o.at[0])
            c.start()
            c.wait()

        return carry

    lax.fori_loop(0, 2, layer, 0)


@jax.jit
def pallas_interleave_layers__sliding_block__moe_arch_mod__prompt_kernel(
    A_x: jax.Array,
    A_wqkv: jax.Array,
    A_wo: jax.Array,
    B_x: jax.Array,
    B_w_r: jax.Array,
    B_w_gate: jax.Array,
    B_w_up: jax.Array,
    B_w_down: jax.Array,
):
    del B_x
    hbm = pl.BlockSpec(memory_space=pl.ANY)
    out = pl.pallas_call(
        _kernel,
        out_shape=jax.ShapeDtypeStruct((S, D), BF16),
        in_specs=[hbm, hbm, hbm, pl.BlockSpec(memory_space=pltpu.VMEM), hbm, hbm, hbm],
        out_specs=hbm,
        scratch_shapes=[
            pltpu.VMEM((S, D), BF16),
            pltpu.VMEM((3 * NG, D, 128), BF16),
            pltpu.VMEM((NG, D, 128), BF16),
            pltpu.VMEM((D, F), BF16),
            pltpu.VMEM((D, F), BF16),
            pltpu.VMEM((F, D), BF16),
            pltpu.VMEM((T // 2, D), U32),
            pltpu.VMEM((T // 2, D), U32),
            pltpu.VMEM((T // 2, 3 * D), U32),
            pltpu.VMEM((T // 2, D), U32),
            pltpu.VMEM((T // 2, D), U32),
            pltpu.VMEM((3 * T // 2, D), U32),
            pltpu.VMEM((D // 2, 3 * T), U32),
            pltpu.VMEM((T // 2, D), U32),
            pltpu.VMEM((T // 2, D), U32),
            pltpu.VMEM((2 * T, D), F32),
            pltpu.VMEM((S // 2, D), U32),
            pltpu.VMEM((8, W + DH, 128), BF16),
            pltpu.VMEM((8, 128), F32),
            pltpu.VMEM((8, 128), jnp.int32),
            pltpu.SemaphoreType.DMA((NB,)),
            pltpu.SemaphoreType.DMA((4 * NG,)),
            pltpu.SemaphoreType.DMA((3,)),
            pltpu.SemaphoreType.DMA((NB,)),
        ],
        compiler_params=pltpu.CompilerParams(vmem_limit_bytes=100 * 2 ** 20),
        name="interleave_layers",
    )(A_x.reshape(S, D), A_wqkv, A_wo, B_w_r, B_w_gate, B_w_up, B_w_down)
    return out.reshape(1, S, D)
```

```python
import functools
import itertools
import math

import jax
import jax.numpy as jnp
import numpy as np
from jax import lax
from jax.experimental import pallas as pl
from jax.experimental.pallas import tpu as pltpu

S = 2048
D = 1024
F = 3584
NH = 32
DH = D // NH
W = 256
T = 256
NB = S // T
NG = D // 128
PS = 4
EPS = float(np.float32(1e-5).astype(jnp.bfloat16))
LOG2E = math.log2(math.e)
QSCALE = float(np.float32(DH ** -0.5).astype(jnp.bfloat16)) * LOG2E
NEG = -1e9 * LOG2E

F32 = jnp.float32
BF16 = jnp.bfloat16
U32 = jnp.uint32
NT_DIMS = (((1,), (1,)), ((), ()))


def _dot(a, b):
    return jnp.dot(a, b, preferred_element_type=F32)


def _dot_nt(a, b):
    return lax.dot_general(a, b, NT_DIMS, preferred_element_type=F32)


def _round(x):
    return x.astype(BF16).astype(F32)


def _after(x, tok):
    return x if tok is None else jnp.where(tok < 0.0, tok, x)


def _row_mean(x, tok=None):
    return _after(jnp.mean(x, axis=-1, keepdims=True), tok)


def _row_scale(x, m):
    mb = _round(m)
    d = x - mb
    v = jnp.mean(d * d, axis=-1, keepdims=True) - (m - mb) * (m - mb)
    v = _round(_round(jnp.maximum(v, 0.0)) + EPS)
    sd = _round(jnp.where(v < jnp.inf, v * lax.rsqrt(v), v))
    return lax.rsqrt(sd * sd)


def _normalise(x, m, inv):
    return (_round(x - _round(m)) * inv).astype(BF16)


def _pack(x):
    return pltpu.bitcast(x, U32)


def _unpack(x):
    return pltpu.bitcast(x, BF16)


def _lane_group(shape):
    return lax.broadcasted_iota(jnp.int32, shape, len(shape) - 1) // DH


def _pick(m, a, b):
    if a is None and b is None:
        return None
    z = jnp.zeros_like(a if a is not None else b)
    return jnp.where(m, a if a is not None else z, b if b is not None else z)


def _regroup(vals, grp):
    st = [_pick(grp % 2 == 0, vals[u], vals[(u + 1) % 4]) for u in range(4)]
    return [_pick(grp < 2, st[(-h) % 4], st[(2 - h) % 4]) for h in range(4)]


def _kernel(x_hbm, wqkv_hbm, wo_hbm, wr_hbm, wg_hbm, wu_hbm, wd_hbm, out_hbm,
            xs, wqkv, wo, wr_ref, wg, wu, wd, hnew, hbuf, qkbuf, qnew, qcur, kwin, vwin, onew, ocur, x1buf, h2buf,
            pbuf, bestv, besti, sem_x, sem_q, sem_w, sem_o):

    def block_rows(i):
        return pl.ds(pl.multiple_of(i * T, T), T)

    def x_copy(i):
        return pltpu.make_async_copy(x_hbm.at[block_rows(i)], xs.at[block_rows(i)], sem_x.at[i])

    def out_copy(i):
        return pltpu.make_async_copy(xs.at[block_rows(i)], out_hbm.at[block_rows(i)], sem_o.at[i])

    def wqkv_copy(c):
        cols = pl.ds(pl.multiple_of(c * 128, 128), 128)
        return pltpu.make_async_copy(wqkv_hbm.at[:, cols], wqkv.at[c], sem_q.at[c])

    wo_copies = [pltpu.make_async_copy(wo_hbm.at[:, c * 128:(c + 1) * 128], wo.at[c], sem_q.at[3 * NG + c])
                 for c in range(NG)] + [pltpu.make_async_copy(wr_hbm, wr_ref, sem_q.at[4 * NG])]
    ffn_copies = [pltpu.make_async_copy(src, dst, sem_w.at[n]) for n, (src, dst) in enumerate(
        [(wg_hbm, wg), (wu_hbm, wu), (wd_hbm, wd)])]
    wqkv_p, wo_p, pbuf_p = wqkv.bitcast(U32), wo.bitcast(U32), pbuf.bitcast(U32)

    def strip(n):
        if isinstance(n, int):
            return (n + 2 * NG) % (3 * NG)
        return jnp.where(n < NG, n + 2 * NG, n - NG)

    x_copy(0).start()
    for c in range(PS):
        wqkv_copy(strip(c)).start()
    pbuf[...] = jnp.zeros_like(pbuf)

    HK = D // 2

    def fold(v):
        out = v[0:8]
        for a in range(1, v.shape[0] // 8):
            out = jnp.maximum(out, v[a * 8:(a + 1) * 8])
        return out[0:1]

    def norm_piece(i, c, n, tok):
        x = xs[pl.ds(pl.multiple_of(i * T + c * n, n), n), :].astype(F32)
        m = _row_mean(x, tok)
        inv = _row_scale(x, m)
        hnew[c * n // 2:(c + 1) * n // 2, :] = _pack(_normalise(x, m, inv))
        return fold(inv)

    def route_piece(i, c, n, tok, stats=None):
        r0 = i * T + c * n
        rows = pl.ds(pl.multiple_of(r0, n), n)
        x1 = x1buf[c * n:(c + 1) * n, :]
        if stats is None:
            m = _row_mean(x1, tok)
            inv = _row_scale(x1, m)
        else:
            m, inv = _after(stats[0], tok), stats[1]
        h2 = _normalise(x1, m, inv)
        h2buf[pl.ds(pl.multiple_of(r0 // 2, n // 2), n // 2), :] = _pack(h2)
        h2 = h2.astype(F32)
        xs[rows, :] = (x1 + h2).astype(BF16)
        r = _round(jnp.sum(h2 * wr_ref[...].astype(F32).reshape(1, D), axis=-1, keepdims=True))
        bv, bi = bestv[...], besti[...]
        sub = lax.broadcasted_iota(jnp.int32, (8, 128), 0) + r0
        for a in range(n // 8):
            ra = jnp.broadcast_to(r[a * 8:(a + 1) * 8], (8, 128))
            better = ra > bv
            bv = jnp.where(better, ra, bv)
            bi = jnp.where(better, sub + a * 8, bi)
        bestv[...] = bv
        besti[...] = bi
        return jnp.abs(bv[0:1])

    def route_stages(b, n):
        tok = yield
        m = _row_mean(x1buf[b * 128:(b + 1) * 128, :], tok)
        tok = yield fold(jnp.abs(m))
        inv = []
        for c in range(2):
            rows = slice(b * 128 + c * 64, b * 128 + (c + 1) * 64)
            inv.append(_row_scale(x1buf[rows, :], _after(m[c * 64:(c + 1) * 64], tok)))
            tok = yield fold(inv[-1])
        inv = jnp.concatenate(inv, axis=0)
        for c in range(128 // n):
            stats = m[c * n:(c + 1) * n], inv[c * n:(c + 1) * n]
            tok = yield route_piece(NB - 2, b * (128 // n) + c, n, tok, stats)[:, 0:1]

    def store_qkv(c, val):
        cols = slice(c % NG * 128, (c % NG + 1) * 128)
        if c < NG:
            qnew[:, cols] = _pack(val)
        elif c < 2 * NG:
            kwin[T:, cols] = _pack(val)
        else:
            vwin[c % NG * 64:(c % NG + 1) * 64, 2 * T:] = _pack(val.T)

    def qkv_rounds():
        for c in [*range(NG), *range(2 * NG, 3 * NG), *range(NG, 2 * NG)]:
            acc = _dot(_unpack(hbuf[:, 0:HK]), _unpack(wqkv_p[c, 0:HK // 2]))
            yield jnp.abs(acc[0:1])
            acc = acc + _dot(_unpack(hbuf[:, HK:]), _unpack(wqkv_p[c, HK // 2:]))
            store_qkv(c, (acc * QSCALE if c < NG else acc).astype(BF16))
            yield jnp.abs(acc[0:1])

    def out_rounds(i):
        rows = block_rows(i)
        ocur[...] = onew[...]
        for c in range(NG):
            cols = slice(c * 128, (c + 1) * 128)
            acc = xs[rows, cols].astype(F32) + _dot(_unpack(ocur[:, 0:HK]), _unpack(wo_p[c, 0:HK // 2]))
            yield jnp.abs(acc[0:1])
            x1buf[0:T, cols] = acc + _dot(_unpack(ocur[:, HK:]), _unpack(wo_p[c, HK // 2:]))
            yield jnp.abs(acc[0:1])

    def final_out_rounds(b):
        rows = slice(S - 2 * T + b * 128, S - 2 * T + (b + 1) * 128)
        src = ocur if b < 2 else onew
        tok = None
        for c in range(NG):
            cols = slice(c * 128, (c + 1) * 128)
            o = src[b % 2 * 64:(b % 2 + 1) * 64, :]
            if tok is not None:
                o = jnp.concatenate([jnp.where(tok < 0.0, jnp.uint32(0), o[0:8]), o[8:]], axis=0)
            x1 = xs[rows, cols].astype(F32) + _dot(_unpack(o), _unpack(wo_p[c]))
            x1buf[b * 128:(b + 1) * 128, cols] = x1
            tok = yield jnp.abs(x1[0:1, 0:1])

    def prologue(l):
        def project(c):
            return _dot(_unpack(hbuf[...]), wqkv[c])

        @pl.when(l == 0)
        def _():
            x_copy(0).wait()
            for c in range(PS, 2 * PS):
                wqkv_copy(strip(c)).start()

        norm_piece(0, 0, T, None)
        hbuf[...] = hnew[...]
        nloop = 3 * NG // PS - 1

        def part(p, carry):
            @pl.when(l == 0)
            def _():
                for c in range(PS):
                    wqkv_copy(strip(p * PS + c)).wait()

                @pl.when(p < nloop - 1)
                def _():
                    for c in range(PS):
                        wqkv_copy(strip((p + 2) * PS + c)).start()

                @pl.when(p >= nloop - 2)
                def _():
                    x_copy(p - nloop + 3).start()

            for c in range(PS):
                c = strip(p * PS + c)
                scale = jnp.where(c < NG, QSCALE, 1.0)
                qkbuf[:, pl.ds(pl.multiple_of(c * 128, 128), 128)] = _pack((project(c) * scale).astype(BF16))
            return carry

        lax.fori_loop(0, nloop, part, 0)

        @pl.when(l == 0)
        def _():
            for c in range(nloop * PS, 3 * NG):
                wqkv_copy(strip(c)).wait()
            x_copy(1).wait()

        for c in range(nloop * PS):
            store_qkv(strip(c), _unpack(qkbuf[:, strip(c) * 128:(strip(c) + 1) * 128]))
        tok = None
        for n in range(PS):
            val = project(strip(nloop * PS + n))
            store_qkv(strip(nloop * PS + n), val.astype(BF16))
            norm_piece(1, n, T // PS, tok)
            tok = jnp.abs(val[0:1, 0:1])

        @pl.when(l == 0)
        def _():
            x_copy(2).wait()
            x_copy(3).start()
            for c in wo_copies:
                c.start()

    def scores(b, g, first_keys):
        lanes = slice(g * 128, (g + 1) * 128)
        if b == 0:
            drows = slice(g * 64, (g + 1) * 64)
            if not first_keys:
                kwin[0:T // 2, lanes] = kwin[T // 2:T, lanes]
                vwin[drows, 0:T] = vwin[drows, T:2 * T]
            kwin[T // 2:T, lanes] = kwin[T:, lanes]
            vwin[drows, T:2 * T] = vwin[drows, 2 * T:]
        grp = _lane_group((DH // 2, 128))
        out = []
        for j in range(4):
            q = qcur[(b * 128 + j * DH) // 2:(b * 128 + (j + 1) * DH) // 2, lanes]
            qbd = jnp.concatenate(
                [jnp.where(grp == (c - j) % 4, q, jnp.zeros_like(q)) for c in range(4)], axis=0)
            lo = max(j, first_keys)
            hi = j + W // DH + 1
            base = T - W + b * 128
            k = kwin[(base + lo * DH) // 2:(base + hi * DH) // 2, lanes]
            out.append((lo, _dot_nt(_unpack(k), _unpack(qbd))))
        return out

    def softmax(ss, first_keys, tok, slot):
        row = lax.broadcasted_iota(jnp.int32, (DH, 128), 0)
        col = lax.broadcasted_iota(jnp.int32, (DH, 128), 1) % DH
        probs, sums = [], []
        for j, (lo, s) in enumerate(ss):
            n = s.shape[0] // DH
            parts = [s[a * DH:(a + 1) * DH] for a in range(n)]
            if lo == j:
                parts[0] = jnp.where(row > col, parts[0], NEG)
            parts[-1] = jnp.where(row <= col, parts[-1], NEG)
            s = jnp.concatenate(parts, axis=0)
            m = jnp.max(s, axis=0, keepdims=True)
            m = _after(m, sums[-1] if sums else tok)
            e = jnp.exp2(s - m)
            sums.append(jnp.sum(e, axis=0, keepdims=True))
            pbuf[slot * 4 + j, 0:n * DH, :] = e.astype(BF16)
            e = pbuf_p[slot * 4 + j, 0:n * DH // 2, :]
            probs.append({lo + a: e[a * DH // 2:(a + 1) * DH // 2] for a in range(n)})
        grp = _lane_group((DH // 2, 128))
        per_head = [[] for _ in range(4)]
        for a in range(first_keys // 4 * 4, 12):
            for h, v in enumerate(_regroup([probs[j].get(a) for j in range(4)], grp)):
                per_head[h].append(v)
        inv = _regroup([1.0 / v for v in sums], _lane_group((1, 128)))
        return [_unpack(jnp.concatenate(p, axis=0)) for p in per_head], inv, sums[-1]

    def values(b, g, first_keys, ps, inv):
        k0 = T - W + b * 128
        t0 = first_keys // 4
        accs = [None] * 4
        for t in range(3):
            if t >= t0:
                for h in range(4):
                    drows = slice((g * 4 + h) * DH // 2, (g * 4 + h + 1) * DH // 2)
                    vt = _unpack(vwin[drows, k0 + t * 128:k0 + (t + 1) * 128])
                    o = _dot(vt, ps[h][(t - t0) * 128:(t - t0 + 1) * 128])
                    accs[h] = o if accs[h] is None else accs[h] + o
            if t == 2:
                outs = [accs[h] * inv[h] for h in range(4)]
                outs = [pltpu.roll(o, (128 - DH * h) % 128, axis=1) if h else o for h, o in enumerate(outs)]
                ot = jnp.concatenate(outs, axis=0)
                onew[b * 64:(b + 1) * 64, g * 128:(g + 1) * 128] = _pack(ot.T.astype(BF16))
            yield

    def step(i, kind):
        groups = [(b, g, max(0, (W - b * 128) // DH) if kind == "first" else 0)
                  for b in range(T // 128) for g in range(NG)]
        ng = len(groups)
        pieces = [[] for _ in range(ng)]
        if kind == "last":
            ocur[...] = onew[...]
            dense = itertools.chain(*[final_out_rounds(b) for b in range(3)])
            per = [2, 1] * (ng // 2)
            for c, n in enumerate([6, 7, 8, 10, 11, 12, 13, 14]):
                pieces[n].append(functools.partial(route_piece, i - 1, c, 32))
        else:
            hbuf[...] = hnew[...]
            ahead = jnp.minimum(i + 2, NB - 1)
            for c in range(8):
                pieces[c * (2 if kind == "first" else 1)].append(functools.partial(norm_piece, ahead, c, T // 8))
            if kind == "first":
                dense, per = qkv_rounds(), [3] * ng
            else:
                dense, per = itertools.chain(out_rounds(i - 1), qkv_rounds()), [4] * ng
                for c in range(8):
                    pieces[7 + c].append(functools.partial(route_piece, i - 1, c, T // 8))

        qcur[...] = qnew[...]
        ss = scores(*groups[0])
        tok, late = None, []
        for n, grp in enumerate(groups):
            nxt = scores(*groups[n + 1]) if n + 1 < ng else None
            ps, inv, tok = softmax(ss, grp[2], tok, n % 2)
            due, late = late, [f(tok[:, 0:1]) for f in pieces[n]]
            for t in (due if kind == "last" else late):
                tok = jnp.maximum(tok, t)
            pv = values(*grp, ps, inv)
            for t in range(4):
                for _ in range((per[n] * (t + 1) + 3) // 4 - (per[n] * t + 3) // 4):
                    td = next(dense)
                    if t == 0 and kind != "first":
                        tok = jnp.maximum(tok, td)
                next(pv, None)
            ss = nxt
        if kind == "last":
            rounds, stages = final_out_rounds(3), route_stages(2, 32)
            next(stages)
            start, done = tok[:, 0:1], None
            for c in range(NG):
                nxt = rounds.send(done)
                if c < NG - 1:
                    done = stages.send(start)
                start = nxt
            route_piece(i - 1, 3, 128, None)

    def ffn():
        bv, bi = bestv[...], besti[...]
        rmax = jnp.max(bv, axis=0, keepdims=True)
        sel = jnp.min(jnp.where(bv == rmax, bi, S - 1))
        tile = sel // 16
        hs = _unpack(h2buf[pl.ds(pl.multiple_of(tile * 8, 8), 8), :])
        y = None
        for c in range(F // 512):
            cols = slice(c * 512, (c + 1) * 512)
            gate = _round(_dot(hs, wg[:, cols]))
            up = _round(_dot(hs, wu[:, cols]))
            act = (_round(gate * jax.nn.sigmoid(gate)) * up).astype(BF16)
            part = jnp.concatenate([_dot(act, wd[cols, a * 128:(a + 1) * 128]) for a in range(NG)], axis=1)
            y = part if y is None else y + part
        y = y * _round(jax.nn.sigmoid(rmax[:, 0:1]))
        hit = lax.broadcasted_iota(jnp.int32, (16, D), 0) + tile * 16 == sel
        return pl.ds(pl.multiple_of(tile * 16, 16), 16), hit, y

    def layer(l, carry):
        bestv[...] = jnp.full((8, 128), -jnp.inf, F32)
        besti[...] = jnp.zeros((8, 128), jnp.int32)

        def emit(i):
            @pl.when(l == 1)
            def _():
                out_copy(i).start()

        prologue(l)
        step(0, "first")

        @pl.when(l == 0)
        def _():
            for c in wo_copies:
                c.wait()
            for i in range(4, NB):
                x_copy(i).start()

        def body(i, c):
            @pl.when(jnp.logical_and(l == 0, i + 2 < NB))
            def _():
                x_copy(i + 2).wait()

            @pl.when(jnp.logical_and(l == 0, i == 2))
            def _():
                for cp in ffn_copies:
                    cp.start()

            step(i, "body")
            emit(i - 1)
            return c

        lax.fori_loop(1, NB - 1, body, 0)
        step(NB - 1, "last")
        emit(NB - 2)
        emit(NB - 1)

        @pl.when(l == 0)
        def _():
            for c in ffn_copies:
                c.wait()

        rows, hit, y = ffn()

        @pl.when(l == 1)
        def _():
            for i in range(NB):
                out_copy(i).wait()

        old = xs[rows, :].astype(F32)
        xs[rows, :] = jnp.where(hit, old + y, old).astype(BF16)

        @pl.when(l == 1)
        def _():
            c = pltpu.make_async_copy(xs.at[rows], out_hbm.at[rows], sem_o.at[0])
            c.start()
            c.wait()

        return carry

    lax.fori_loop(0, 2, layer, 0)


@jax.jit
def pallas_interleave_layers__sliding_block__moe_arch_mod__prompt_kernel(
    A_x: jax.Array,
    A_wqkv: jax.Array,
    A_wo: jax.Array,
    B_x: jax.Array,
    B_w_r: jax.Array,
    B_w_gate: jax.Array,
    B_w_up: jax.Array,
    B_w_down: jax.Array,
):
    del B_x
    hbm = pl.BlockSpec(memory_space=pl.ANY)
    out = pl.pallas_call(
        _kernel,
        out_shape=jax.ShapeDtypeStruct((S, D), BF16),
        in_specs=[hbm] * 7,
        out_specs=hbm,
        scratch_shapes=[
            pltpu.VMEM((S, D), BF16),
            pltpu.VMEM((3 * NG, D, 128), BF16),
            pltpu.VMEM((NG, D, 128), BF16),
            pltpu.VMEM((D,), BF16),
            pltpu.VMEM((D, F), BF16),
            pltpu.VMEM((D, F), BF16),
            pltpu.VMEM((F, D), BF16),
            pltpu.VMEM((T // 2, D), U32),
            pltpu.VMEM((T // 2, D), U32),
            pltpu.VMEM((T // 2, 3 * D), U32),
            pltpu.VMEM((T // 2, D), U32),
            pltpu.VMEM((T // 2, D), U32),
            pltpu.VMEM((3 * T // 2, D), U32),
            pltpu.VMEM((D // 2, 3 * T), U32),
            pltpu.VMEM((T // 2, D), U32),
            pltpu.VMEM((T // 2, D), U32),
            pltpu.VMEM((2 * T, D), F32),
            pltpu.VMEM((S // 2, D), U32),
            pltpu.VMEM((8, W + DH, 128), BF16),
            pltpu.VMEM((8, 128), F32),
            pltpu.VMEM((8, 128), jnp.int32),
            pltpu.SemaphoreType.DMA((NB,)),
            pltpu.SemaphoreType.DMA((4 * NG + 1,)),
            pltpu.SemaphoreType.DMA((3,)),
            pltpu.SemaphoreType.DMA((NB,)),
        ],
        compiler_params=pltpu.CompilerParams(vmem_limit_bytes=100 * 2 ** 20),
        name="interleave_layers",
    )(A_x.reshape(S, D), A_wqkv, A_wo, B_w_r, B_w_gate, B_w_up, B_w_down)
    return out.reshape(1, S, D)
```
